```python
import os as _os
_os.environ.setdefault("JAX_PLATFORMS", "cpu")
import jax
import jax.numpy as jnp

def _softmax(x, axis=-1):
    return jax.nn.softmax(x, axis=axis)
def _gelu(x):
    return jax.nn.gelu(x, approximate=True)
def _silu(x):
    return jax.nn.silu(x)
def _sigmoid(x):
    return jax.nn.sigmoid(x)
def _layernorm(x, axis=-1, eps=1e-5):
    m = jnp.mean(x, axis=axis, keepdims=True)
    v = jnp.var(x, axis=axis, keepdims=True)
    return (x - m) / jnp.sqrt(v + eps)
def _scatter_add(tgt, idx, src, axis=0):
    return tgt.at[idx].add(src)
def _segment_sum(src, seg, n):
    return jax.ops.segment_sum(src, seg, n)
class _Rng:
    def __init__(self, key):
        self._k = key
    def _next(self):
        self._k, sub = jax.random.split(self._k)
        return sub
    def normal(self, shape):
        return jax.random.normal(self._next(), shape, dtype=jnp.bfloat16)
    def randint(self, lo, hi, shape):
        return jax.random.randint(self._next(), shape, lo, hi, dtype=jnp.int32)
    def uniform(self, shape, lo=0.0, hi=1.0):
        return jax.random.uniform(self._next(), shape, jnp.bfloat16, lo, hi)
    def permutation(self, n):
        return jax.random.permutation(self._next(), n)


kernel_name = 'concat_heads__grouped_kv_mqa__sliding_block__prompt'

def setup_inputs():
    _rng = _Rng(jax.random.key(int.from_bytes(__import__("os").urandom(4), "little")))
    _w = (lambda a: (lambda t: t.astype(jnp.bfloat16) if jnp.issubdtype(t.dtype, jnp.floating) else t)(jnp.asarray(a)))
    def _A_setup():
        B, S, D, H = 1, 2048, 1024, 32
        Dh = D // H
        return {
            "x": _w((lambda *s: _rng.normal(s) * 0.05)(B, S, D)),
            "wq": _w((lambda *s: _rng.normal(s) * 1.6)(D, H * Dh)),
            "wk": _w((lambda *s: _rng.normal(s) * 1.6)(D, Dh)),
            "wv": _w((lambda *s: _rng.normal(s) * 0.1)(D, Dh)),
            "wo": _w((lambda *s: _rng.normal(s) * 0.1)(H * Dh, D)),
        }
    _A_in = _A_setup()

    def _B_setup():
        B, S, D = 1, 2048, 1024
        return {
            "x": _w((lambda *s: _rng.normal(s) * 0.2)(B, S, D)),
            "wqkv": _w((lambda *s: _rng.normal(s) * 0.2)(D, 3 * D)),
            "wo": _w((lambda *s: _rng.normal(s) * 0.05)(D, D)),
        }
    _B_in = _B_setup()

    return {
        "A_x": _A_in["x"],
        "A_wq": _A_in["wq"],
        "A_wk": _A_in["wk"],
        "A_wv": _A_in["wv"],
        "A_wo": _A_in["wo"],
        "B_x": _B_in["x"],
        "B_wqkv": _B_in["wqkv"],
        "B_wo": _B_in["wo"],
    }

def reference(A_x, A_wq, A_wk, A_wv, A_wo, B_x, B_wqkv, B_wo):
    def _A_ref(x, wq, wk, wv, wo):
        B, S, D = x.shape
        H = 32
        Dh = D // H
        q = (lambda x, *d: x.transpose(*d))((x @ wq).reshape(B, S, H, Dh), 0, 2, 1, 3)
        k = x @ wk
        v = x @ wv
        scores = jnp.einsum("bhqd,bkd->bhqk", q, k) * (Dh ** -0.5)
        p = _softmax(scores, axis=-1)
        o = jnp.einsum("bhqk,bkd->bhqd", p, v)
        return (lambda x, *d: x.transpose(*d))(o, 0, 2, 1, 3).reshape(B, S, H * Dh) @ wo

    def _B_ref(x, wqkv, wo):
        B, S, D = x.shape
        H = 32; Dh = D // H; W = 256
        qkv = (lambda x, *d: x.transpose(*d))((x @ wqkv).reshape(B, S, 3, H, Dh), 2, 0, 3, 1, 4)
        q, k, v = qkv[0], qkv[1], qkv[2]
        scores = jnp.einsum("bhqd,bhkd->bhqk", q, k) * (Dh ** -0.5)
        idx = jnp.arange(S)
        mask = (idx[:, None] - idx[None, :] >= 0) & (idx[:, None] - idx[None, :] < W)
        scores = jnp.where(mask[None, None], scores, -1e9)
        p = _softmax(scores, axis=-1)
        o = jnp.einsum("bhqk,bhkd->bhqd", p, v)
        return (lambda x, *d: x.transpose(*d))(o, 0, 2, 1, 3).reshape(B, S, D) @ wo

    a = _A_ref(A_x, A_wq, A_wk, A_wv, A_wo)
    b = _B_ref(B_x, B_wqkv, B_wo)
    return jnp.concatenate([a, b], axis=-1)
```

```python
import jax
import jax.numpy as jnp
import numpy as np
from jax import lax
import jax.experimental.pallas as pl
import jax.experimental.pallas.tpu as pltpu

_BF = jnp.bfloat16
_F32 = jnp.float32

_S = 2048
_D = 1024
_H = 32
_DH = 32
_W = 256
_QB = 512
_NB = _S // _QB
_T = 128
_CH = 128
_LOG2E = 1.4426950408889634
_QSCALE = (_DH ** -0.5) * _LOG2E
_NEG = -1e9 * _LOG2E

_TT = (((0,), (1,)), ((), ()))
_TN = (((0,), (0,)), ((), ()))


def _dot(a, b, dims=(((1,), (0,)), ((), ()))):
    return lax.dot_general(a, b, dims, preferred_element_type=_F32)


def _colmax8(s):
    r, n = s.shape
    return jnp.max(s.reshape(r // 8, 8, n), axis=0)


def _normalize(o):
    inv = 1.0 / o[32:40]
    return jnp.concatenate([o[8 * r:8 * r + 8] * inv for r in range(4)], axis=0)


def _kernel(xa_hbm, wqa_hbm, wka_ref, wva_ref, woa_hbm, xb_hbm, wqkvb_hbm, wob_hbm,
            out_hbm,
            xa, xb, wqa, wqkvb, wo, wkva, qta, ka, vta, sa, ot, qtb, kb, vtb, sb, ostage,
            in_sem, out_sem):
    c_wqa = pltpu.make_async_copy(wqa_hbm, wqa, in_sem.at[0])
    c_xa = [pltpu.make_async_copy(xa_hbm.at[0, pl.ds(b * _QB, _QB)],
                                  xa.at[pl.ds(b * _QB, _QB)], in_sem.at[1 + b])
            for b in range(_NB)]
    c_woa = pltpu.make_async_copy(woa_hbm, wo.at[0], in_sem.at[5])
    c_xb = pltpu.make_async_copy(xb_hbm.at[0], xb, in_sem.at[6])
    c_wqkvb = pltpu.make_async_copy(wqkvb_hbm, wqkvb, in_sem.at[7])
    c_wob = pltpu.make_async_copy(wob_hbm, wo.at[1], in_sem.at[8])

    c_wqa.start()
    c_xa[0].start()
    for b in range(1, _NB):
        c_xa[b].start()

    wkva[...] = jnp.concatenate([wka_ref[...], wva_ref[...]], axis=1)
    ones16 = jnp.ones((16, _T), _BF)

    c_wqa.wait()
    for b in range(_NB):
        c_xa[b].wait()
        if b == 0:
            c_xb.start()
            c_wqkvb.start()
            c_woa.start()
            c_wob.start()

    def a_proj(b, carry):
        r0 = pl.multiple_of(b * _QB, _QB)
        x = xa[pl.ds(r0, _QB), :]
        kv = _dot(wkva[...], x, _TT)
        vta[:, pl.ds(r0, _QB)] = kv[32:64].astype(_BF)
        ka[pl.ds(r0, _QB), :] = kv[0:32].T.astype(_BF)
        q = _dot(wqa[...], x, _TT)
        qta[:, pl.ds(r0, _QB)] = (q * _QSCALE).astype(_BF)
        return carry

    lax.fori_loop(0, _NB, a_proj, 0)

    n_c = _S // _CH

    def a_qk_chunk(q, slot, c, mx):
        s = _dot(ka[c * _CH:(c + 1) * _CH, :], q)
        sa[slot, c * _CH:(c + 1) * _CH, :] = s
        mc = _colmax8(s)
        return mc if mx is None else jnp.maximum(mx, mc)

    def a_pv_chunk(slot, c, m, acc):
        p = jnp.exp2(sa[slot, c * _CH:(c + 1) * _CH, :] - m).astype(_BF)
        lhs = jnp.concatenate([vta[:, c * _CH:(c + 1) * _CH], ones16], axis=0)
        pv = _dot(lhs, p)
        return pv if acc is None else acc + pv

    def a_q_tile(t):
        h0 = pl.multiple_of((t % _H) * _DH, _DH)
        r0 = pl.multiple_of((t // _H) * _QB, _QB)
        return qta[pl.ds(h0, _DH), pl.ds(r0, _QB)]

    q = a_q_tile(0)
    mx = None
    for c in range(n_c):
        mx = a_qk_chunk(q, 0, c, mx)
    m0 = jnp.max(mx, axis=0, keepdims=True)

    n_steps = _NB * _H

    def a_body(it, m):
        for u in range(2):
            t = it * 2 + u
            qn = a_q_tile(jnp.minimum(t + 1, n_steps - 1))
            mx = None
            acc = None
            for c in range(n_c):
                mx = a_qk_chunk(qn, 1 - u, c, mx)
                acc = a_pv_chunk(u, c, m, acc)
            h0 = pl.multiple_of((t % _H) * _DH, _DH)
            r0 = pl.multiple_of((t // _H) * _QB, _QB)
            ot[0, pl.ds(h0, _DH), pl.ds(r0, _QB)] = _normalize(acc).astype(_BF)
            m = jnp.max(mx, axis=0, keepdims=True)
        return m

    lax.fori_loop(0, n_steps // 2, a_body, m0)

    c_xb.wait()
    c_wqkvb.wait()

    def b_proj_qv(i, carry):
        b = i // 2
        j = i % 2
        r0 = pl.multiple_of(b * _QB, _QB)
        c0 = pl.multiple_of(j * 2 * _D, _D)
        y = _dot(wqkvb[:, pl.ds(c0, _D)], xb[pl.ds(r0, _QB), :], _TT)
        scale = jnp.where(j == 0, _QSCALE, 1.0)
        qvb = (y * scale).astype(_BF)

        @pl.when(j == 0)
        def _():
            qtb[:, pl.ds(r0, _QB)] = qvb

        @pl.when(j == 1)
        def _():
            vtb[:, pl.ds(r0, _QB)] = qvb
        return carry

    lax.fori_loop(0, 2 * _NB, b_proj_qv, 0)

    def b_proj_k(b, carry):
        r0 = pl.multiple_of(b * _QB, _QB)
        kb[pl.ds(r0, _QB), :] = _dot(xb[pl.ds(r0, _QB), :], wqkvb[:, _D:2 * _D]).astype(_BF)
        return carry

    lax.fori_loop(0, _NB, b_proj_k, 0)

    dd = (lax.broadcasted_iota(jnp.int32, (_T, _T), 0)
          - lax.broadcasted_iota(jnp.int32, (_T, _T), 1))

    def b_build_q(i, g):
        q = qtb[g * _T:(g + 1) * _T, pl.ds(pl.multiple_of(i * _T, _T), _T)]
        q32 = pltpu.bitcast(q, jnp.uint32)
        z = jnp.zeros((16, _T), jnp.uint32)
        cols = [jnp.concatenate([q32[16 * r:16 * r + 16] if r == j else z for r in range(4)], axis=0)
                for j in range(4)]
        return pltpu.bitcast(jnp.concatenate(cols, axis=1), _BF)

    def b_qk(i, g, slot, tiles):
        qb = b_build_q(i, g)
        mx = None
        for t in tiles:
            kv0 = pl.multiple_of((i - 2 + t) * _T, _T)
            s = _dot(kb[pl.ds(kv0, _T), g * _T:(g + 1) * _T], qb)
            if t != 1:
                msk = (dd > 0) if t == 0 else (dd <= 0)
                s = jnp.concatenate(
                    [jnp.where(msk, s[:, j * _T:(j + 1) * _T], _NEG) for j in range(4)], axis=1)
            sb[slot, t * _T:(t + 1) * _T, :] = s
            mc = _colmax8(s)
            mx = mc if mx is None else jnp.maximum(mx, mc)
        return jnp.max(mx, axis=0, keepdims=True)

    def b_pv(i, g, slot, m, tiles):
        t0, nt = tiles[0], len(tiles)
        kv0 = pl.multiple_of((i - 2 + t0) * _T, _T)
        p = jnp.exp2(sb[slot, t0 * _T:(t0 + nt) * _T, :] - m).astype(_BF)
        ones = jnp.ones((16, nt * _T), _BF)
        for j in range(4):
            h = 4 * g + j
            lhs = jnp.concatenate([vtb[h * _DH:(h + 1) * _DH, pl.ds(kv0, nt * _T)], ones], axis=0)
            o = _dot(lhs, p[:, j * _T:(j + 1) * _T])
            ot[1, h * _DH:(h + 1) * _DH, pl.ds(pl.multiple_of(i * _T, _T), _T)] = (
                _normalize(o).astype(_BF))

    n_g = _H // 4
    n_t = _S // _T
    steps = ([(0, g, [2]) for g in range(n_g)] + [(1, g, [1, 2]) for g in range(n_g)]
             + [(2, 0, [0, 1, 2])])
    m = b_qk(steps[0][0], steps[0][1], 0, steps[0][2])
    for n in range(2 * n_g):
        i, g, tiles = steps[n]
        i2, g2, tiles2 = steps[n + 1]
        m2 = b_qk(i2, g2, (n + 1) % 2, tiles2)
        b_pv(i, g, n % 2, m, tiles)
        m = m2

    def b_body(i, m):
        for g in range(n_g):
            if g + 1 < n_g:
                m2 = b_qk(i, g + 1, (g + 1) % 2, [0, 1, 2])
            else:
                m2 = b_qk(jnp.minimum(i + 1, n_t - 1), 0, (g + 1) % 2, [0, 1, 2])
            b_pv(i, g, g % 2, m, [0, 1, 2])
            m = m2
        return m

    lax.fori_loop(2, n_t, b_body, m)

    c_woa.wait()
    c_wob.wait()

    def out_copy(n):
        ab = n // _NB
        b = n % _NB
        return pltpu.make_async_copy(
            ostage.at[n],
            out_hbm.at[0, pl.ds(pl.multiple_of(b * _QB, _QB), _QB),
                       pl.ds(pl.multiple_of(ab * _D, _D), _D)],
            out_sem.at[n])

    def o_proj(n, carry):
        ab = n // _NB
        r0 = pl.multiple_of((n % _NB) * _QB, _QB)
        y = _dot(ot[ab, :, pl.ds(r0, _QB)], wo[ab], _TN)
        ostage[n] = y.astype(_BF)
        out_copy(n).start()
        return carry

    lax.fori_loop(0, 2 * _NB, o_proj, 0)
    for n in range(2 * _NB):
        out_copy(n).wait()


@jax.jit
def pallas_concat_heads__grouped_kv_mqa__sliding_block__prompt_kernel(
    A_x: jax.Array,
    A_wq: jax.Array,
    A_wk: jax.Array,
    A_wv: jax.Array,
    A_wo: jax.Array,
    B_x: jax.Array,
    B_wqkv: jax.Array,
    B_wo: jax.Array,
):
    hbm = pl.BlockSpec(memory_space=pl.ANY)
    vmem = pl.BlockSpec(memory_space=pltpu.VMEM)
    return pl.pallas_call(
        _kernel,
        out_shape=jax.ShapeDtypeStruct((1, _S, 2 * _D), _BF),
        in_specs=[hbm, hbm, vmem, vmem, hbm, hbm, hbm, hbm],
        out_specs=hbm,
        scratch_shapes=[
            pltpu.VMEM((_S, _D), _BF),
            pltpu.VMEM((_S, _D), _BF),
            pltpu.VMEM((_D, _D), _BF),
            pltpu.VMEM((_D, 3 * _D), _BF),
            pltpu.VMEM((2, _D, _D), _BF),
            pltpu.VMEM((_D, 2 * _DH), _BF),
            pltpu.VMEM((_D, _S), _BF),
            pltpu.VMEM((_S, _DH), _BF),
            pltpu.VMEM((_DH, _S), _BF),
            pltpu.VMEM((2, _S, _QB), _F32),
            pltpu.VMEM((2, _D, _S), _BF),
            pltpu.VMEM((_D, _S), _BF),
            pltpu.VMEM((_S, _D), _BF),
            pltpu.VMEM((_D, _S), _BF),
            pltpu.VMEM((2, 3 * _T, 4 * _T), _F32),
            pltpu.VMEM((2 * _NB, _QB, _D), _BF),
            pltpu.SemaphoreType.DMA((9,)),
            pltpu.SemaphoreType.DMA((2 * _NB,)),
        ],
        compiler_params=pltpu.CompilerParams(vmem_limit_bytes=100 * 1024 * 1024),
    )(A_x, A_wq, A_wk, A_wv, A_wo, B_x, B_wqkv, B_wo)
```

```python
import jax
import jax.numpy as jnp
from jax import lax
import jax.experimental.pallas as pl
import jax.experimental.pallas.tpu as pltpu

_BF = jnp.bfloat16
_F32 = jnp.float32

_S = 2048
_D = 1024
_H = 32
_DH = 32
_QB = 512
_NB = _S // _QB
_T = 128
_LOG2E = 1.4426950408889634
_QSCALE = (_DH ** -0.5) * _LOG2E
_NEG = -1e9 * _LOG2E

_A_UNROLL = 8
_B_UNROLL = 6

_NN = (((1,), (0,)), ((), ()))
_TT = (((0,), (1,)), ((), ()))
_NT = (((1,), (1,)), ((), ()))


def _dot(a, b, dims=_NN):
    return lax.dot_general(a, b, dims, preferred_element_type=_F32)


def _ds(i, size):
    if isinstance(i, int):
        return pl.ds(i * size, size)
    return pl.ds(pl.multiple_of(i * size, size), size)


def _colmax8(s):
    r, n = s.shape
    return jnp.max(s.reshape(r // 8, 8, n), axis=0)


def _colmax(mx):
    return jnp.max(mx, axis=0, keepdims=True)


def _colsum8(l, p, extra_latency):
    n = p.shape[0] // 8
    for k in range(n):
        r = n - 1 - k
        l = p[8 * r:8 * r + 8] if l is None else l + p[8 * r:8 * r + 8]
        if extra_latency and k % 2 == 1 and k < n - 2:
            l = jnp.abs(l)
    return l


def _kernel(xa_hbm, wqa_hbm, wkta_hbm, wvta_hbm, woa_hbm, xb_hbm, wqkvb_hbm, wob_hbm,
            out_hbm,
            xa, xb, wqa, wkva, wqkvb, wt, wo, qta, ka, vta, sa, qvtb, kb, sb,
            ot, obuf, ostage, in_sem, out_sem):
    half = _D // 2
    c_wk = pltpu.make_async_copy(wkta_hbm, wkva.at[pl.ds(0, _DH)], in_sem.at[0])
    c_wv = pltpu.make_async_copy(wvta_hbm, wkva.at[pl.ds(_DH, _DH)], in_sem.at[0])
    c_x0 = pltpu.make_async_copy(xa_hbm.at[0, pl.ds(0, _QB)], xa.at[pl.ds(0, _QB)], in_sem.at[1])
    c_wq = [pltpu.make_async_copy(wqa_hbm.at[:, pl.ds(j * half, half)],
                                  wqa.at[:, pl.ds(j * half, half)], in_sem.at[2 + j])
            for j in range(2)]
    c_x1 = pltpu.make_async_copy(xa_hbm.at[0, pl.ds(_QB, _S - _QB)],
                                 xa.at[pl.ds(_QB, _S - _QB)], in_sem.at[4])
    c_xb = pltpu.make_async_copy(xb_hbm.at[0], xb, in_sem.at[5])
    c_wqkvb = pltpu.make_async_copy(wqkvb_hbm, wqkvb, in_sem.at[6])
    c_woa = pltpu.make_async_copy(woa_hbm, wo.at[0], in_sem.at[7])
    c_wob = pltpu.make_async_copy(wob_hbm, wo.at[1], in_sem.at[7])
    for c in (c_wk, c_wv, c_x0, c_wq[0], c_wq[1], c_x1, c_xb, c_wqkvb, c_woa, c_wob):
        c.start()

    def a_proj_kv(x, rows):
        kv = _dot(wkva[...], x, _NT)
        ka[rows, :] = kv[0:_DH].T.astype(_BF)
        vta[:, rows] = kv[_DH:2 * _DH].astype(_BF).astype(_F32)

    def a_proj_q(x, rows, cols):
        qta[cols, rows] = (_dot(wqa[:, cols], x, _TT) * _QSCALE).astype(_BF)

    c_wk.wait()
    c_wv.wait()
    c_x0.wait()
    x0 = xa[0:_QB, :]
    a_proj_kv(x0, pl.ds(0, _QB))
    for j in range(2):
        c_wq[j].wait()
        a_proj_q(x0, pl.ds(0, _QB), pl.ds(j * half, half))
    c_x1.wait()

    def a_proj(b, carry):
        rows = _ds(b, _QB)
        x = xa[rows, :]
        a_proj_kv(x, rows)
        a_proj_q(x, rows, pl.ds(0, _D))
        return carry

    lax.fori_loop(1, _NB, a_proj, 0)

    n_c = _S // _T
    n_steps = _NB * _H

    def a_pos(t):
        if isinstance(t, int):
            return _ds(t % _H, _DH), _ds(t // _H, _QB)
        return _ds(t & (_H - 1), _DH), _ds(lax.shift_right_logical(t, 5), _QB)

    def a_q(t):
        rows, cols = a_pos(t)
        return qta[rows, cols]

    def a_scores(q, slot, c, mx):
        s = _dot(ka[c * _T:(c + 1) * _T, :], q)
        sa[slot, c * _T:(c + 1) * _T, :] = s
        mc = _colmax8(s)
        return mc if mx is None else jnp.maximum(mx, mc)

    def a_pv(slot, c, m, acc, l):
        p = jnp.exp2(sa[slot, c * _T:(c + 1) * _T, :] - m)
        l = _colsum8(l, p, True)
        zero = (((l[:, 0:128] + l[:, 128:256]) + l[:, 256:384]) + l[:, 384:512]) * 0.0
        vt = vta[:, c * _T:(c + 1) * _T]
        vt = jnp.concatenate([vt[0:8] + zero, vt[8:16], vt[16:24], vt[24:32]], axis=0)
        pv = _dot(vt, p.astype(_BF))
        return (pv if acc is None else acc + pv), l

    def a_step(t, slot, m, mx, n_ahead):
        acc = l = m_next = None
        if n_ahead >= 1:
            q1 = a_q(t + 1)
        for c in range(n_c):
            if c + 1 < n_c:
                if n_ahead >= 1:
                    mx = a_scores(q1, 1 - slot, c + 1, mx)
                if c + 2 == n_c:
                    m_next = _colmax(mx) if n_ahead >= 1 else None
                    mx = None
                    if n_ahead >= 2:
                        q2 = a_q(t + 2)
            elif n_ahead >= 2:
                mx = a_scores(q2, slot, 0, mx)
            acc, l = a_pv(slot, c, m, acc, l)
        rows, cols = a_pos(t)
        ot[0, rows, cols] = (acc * (1.0 / jnp.sum(l, axis=0, keepdims=True))).astype(_BF)
        return m_next, mx

    c_wqkvb.wait()
    wt[0] = wqkvb[:, 0:_D].T

    q = a_q(0)
    mx = None
    for c in range(n_c):
        mx = a_scores(q, 0, c, mx)
    m = _colmax(mx)
    mx = a_scores(a_q(1), 1, 0, None)

    def a_body(it, carry):
        m, mx = carry
        for u in range(_A_UNROLL):
            m, mx = a_step(it * _A_UNROLL + u, u % 2, m, mx, 2)
        return m, mx

    n_it = (n_steps - 2) // _A_UNROLL
    m, mx = lax.fori_loop(0, n_it, a_body, (m, mx))
    c_xb.wait()
    wt[1] = wqkvb[:, 2 * _D:3 * _D].T
    for t in range(n_it * _A_UNROLL, n_steps):
        m, mx = a_step(t, t % 2, m, mx, min(n_steps - 1 - t, 2))

    def b_proj_qv(b, carry):
        rows = _ds(b, _QB)
        x = xb[rows, :]
        qvtb[0, :, rows] = (_dot(wt[0], x, _NT) * _QSCALE).astype(_BF)
        qvtb[1, :, rows] = _dot(wt[1], x, _NT).astype(_BF)
        return carry

    lax.fori_loop(0, _NB, b_proj_qv, 0)

    def b_proj_k(b, carry):
        rows = _ds(b, 2 * _QB)
        kb[rows, :] = _dot(xb[rows, :], wqkvb[:, _D:2 * _D]).astype(_BF)
        return carry

    lax.fori_loop(0, _NB // 2, b_proj_k, 0)

    dd = (lax.broadcasted_iota(jnp.int32, (_T, _T), 0)
          - lax.broadcasted_iota(jnp.int32, (_T, _T), 1))

    def o_untranspose(n, slot):
        obuf[slot] = ot[n // _NB, :, _ds(n % _NB, _QB)].T

    o_untranspose(0, 0)

    def b_q(i, g):
        q = pltpu.bitcast(qvtb[0, g * _T:(g + 1) * _T, _ds(i, _T)], jnp.uint32)
        z = jnp.zeros((16, _T), jnp.uint32)
        cols = [jnp.concatenate([q[16 * r:16 * r + 16] if r == j else z for r in range(4)], axis=0)
                for j in range(4)]
        return pltpu.bitcast(jnp.concatenate(cols, axis=1), _BF)

    def b_scores(q, i, g, slot, t, mx):
        s = _dot(kb[_ds(i - 2 + t, _T), g * _T:(g + 1) * _T], q)
        if t != 1:
            keep = dd > 0 if t == 0 else dd <= 0
            s = jnp.concatenate(
                [jnp.where(keep, s[:, j * _T:(j + 1) * _T], _NEG) for j in range(4)], axis=1)
        sb[slot, t * _T:(t + 1) * _T, :] = s
        mc = _colmax8(s)
        return mc if mx is None else jnp.maximum(mx, mc)

    def b_pv(i, g, slot, t, m, acc, l):
        p = jnp.exp2(sb[slot, t * _T:(t + 1) * _T, :] - m)
        l = _colsum8(l, p, False)
        out = []
        for j in range(4):
            h = 4 * g + j
            lanes = slice(j * _T, (j + 1) * _T)
            v = pltpu.bitcast(qvtb[1, h * _DH:(h + 1) * _DH, _ds(i - 2 + t, _T)], jnp.uint32)
            zero = pltpu.bitcast(l[:, lanes] * 0.0, jnp.uint32)
            v = pltpu.bitcast(jnp.concatenate([v[0:8] | zero, v[8:16]], axis=0), _BF)
            o = _dot(v, p[:, lanes].astype(_BF))
            out.append(o if acc is None else acc[j] + o)
        return out, l

    def b_step(cur, nxt, n, m, l_prev):
        i, g, tiles = cur
        i2, g2, tiles2 = nxt if nxt is not None else (None, None, ())
        if tiles2:
            q = b_q(i2, g2)
        mx = acc = None
        l = None if l_prev is None else l_prev * 0.0
        for k in range(max(len(tiles), len(tiles2))):
            if k < len(tiles2):
                mx = b_scores(q, i2, g2, (n + 2) % 4, tiles2[k], mx)
            if k < len(tiles):
                acc, l = b_pv(i, g, n % 4, tiles[k], m, acc, l)
        inv = 1.0 / jnp.sum(l, axis=0, keepdims=True)
        for j in range(4):
            h = 4 * g + j
            ot[1, h * _DH:(h + 1) * _DH, _ds(i, _T)] = (
                acc[j] * inv[:, j * _T:(j + 1) * _T]).astype(_BF)
        return (_colmax(mx) if tiles2 else None), l

    n_g = _H // 4
    n_t = _S // _T
    full = (0, 1, 2)
    head = ([(0, g, (2,)) for g in range(n_g)] + [(1, g, (1, 2)) for g in range(n_g)]
            + [(2, 0, full), (2, 1, full)])
    m_a = _colmax(b_scores(b_q(0, 0), 0, 0, 0, 2, None))
    m_b = _colmax(b_scores(b_q(0, 1), 0, 1, 1, 2, None))
    l = None
    for n in range(2 * n_g):
        m_c, l = b_step(head[n], head[n + 2], n, m_a, l)
        m_a, m_b = m_b, m_c

    def b_tile(i, ms, l, last):
        m_a, m_b = ms
        for g in range(n_g):
            if g + 2 < n_g:
                nxt = (i, g + 2, full)
            else:
                nxt = None if last else (i + 1, g + 2 - n_g, full)
            m_c, l = b_step((i, g, full), nxt, g, m_a, l)
            m_a, m_b = m_b, m_c
        return (m_a, m_b), l

    def b_body(it, ms):
        l = None
        for u in range(_B_UNROLL):
            ms, l = b_tile(2 + it * _B_UNROLL + u, ms, l, False)
        return ms

    n_it = (n_t - 3) // _B_UNROLL
    ms = lax.fori_loop(0, n_it, b_body, (m_a, m_b))
    l = None
    for i in range(2 + n_it * _B_UNROLL, n_t):
        ms, l = b_tile(i, ms, l, i == n_t - 1)

    c_woa.wait()
    c_wob.wait()
    qs = _QB // 2

    def out_copy(n, j, k):
        return pltpu.make_async_copy(
            ostage.at[n, pl.ds(j * qs, qs), pl.ds(k * half, half)],
            out_hbm.at[0, _ds(n % _NB * 2 + j, qs), _ds(n // _NB * 2 + k, half)],
            out_sem)

    def o_proj(it, carry):
        for u in range(2):
            n = it * 2 + u
            o_untranspose(jnp.minimum(n + 1, 2 * _NB - 1), 1 - u)
            for j in range(2):
                o = obuf[u, j * qs:(j + 1) * qs, :]
                for k in range(2):
                    y = _dot(o, wo[n // _NB, :, k * half:(k + 1) * half])
                    ostage[n, j * qs:(j + 1) * qs, k * half:(k + 1) * half] = y.astype(_BF)
                    out_copy(n, j, k).start()
        return carry

    lax.fori_loop(0, _NB, o_proj, 0)
    for n in range(2 * _NB):
        for j in range(2):
            for k in range(2):
                out_copy(n, j, k).wait()


@jax.jit
def pallas_concat_heads__grouped_kv_mqa__sliding_block__prompt_kernel(
    A_x: jax.Array,
    A_wq: jax.Array,
    A_wk: jax.Array,
    A_wv: jax.Array,
    A_wo: jax.Array,
    B_x: jax.Array,
    B_wqkv: jax.Array,
    B_wo: jax.Array,
):
    hbm = pl.BlockSpec(memory_space=pl.ANY)
    return pl.pallas_call(
        _kernel,
        out_shape=jax.ShapeDtypeStruct((1, _S, 2 * _D), _BF),
        in_specs=[hbm] * 8,
        out_specs=hbm,
        scratch_shapes=[
            pltpu.VMEM((_S, _D), _BF),
            pltpu.VMEM((_S, _D), _BF),
            pltpu.VMEM((_D, _D), _BF),
            pltpu.VMEM((2 * _DH, _D), _BF),
            pltpu.VMEM((_D, 3 * _D), _BF),
            pltpu.VMEM((2, _D, _D), _BF),
            pltpu.VMEM((2, _D, _D), _BF),
            pltpu.VMEM((_D, _S), _BF),
            pltpu.VMEM((_S, _DH), _BF),
            pltpu.VMEM((_DH, _S), _F32),
            pltpu.VMEM((2, _S, _QB), _F32),
            pltpu.VMEM((2, _D, _S), _BF),
            pltpu.VMEM((_S, _D), _BF),
            pltpu.VMEM((4, 3 * _T, 4 * _T), _F32),
            pltpu.VMEM((2, _D, _S), _BF),
            pltpu.VMEM((2, _QB, _D), _BF),
            pltpu.VMEM((2 * _NB, _QB, _D), _BF),
            pltpu.SemaphoreType.DMA((8,)),
            pltpu.SemaphoreType.DMA(()),
        ],
        compiler_params=pltpu.CompilerParams(vmem_limit_bytes=100 * 1024 * 1024),
    )(A_x, A_wq, A_wk.T, A_wv.T, A_wo, B_x, B_wqkv, B_wo)
```
